```python
import jax
import jax.numpy as jnp

def _softmax(x, axis=-1):
    return jax.nn.softmax(x, axis=axis)

def _gelu(x):
    return jax.nn.gelu(x, approximate=True)

def _silu(x):
    return jax.nn.silu(x)

def _sigmoid(x):
    return jax.nn.sigmoid(x)

def _layernorm(x, axis=-1, eps=1e-05):
    m = jnp.mean(x, axis=axis, keepdims=True)
    v = jnp.var(x, axis=axis, keepdims=True)
    return (x - m) / jnp.sqrt(v + eps)

def _scatter_add(tgt, idx, src, axis=0):
    return tgt.at[idx].add(src)

def _segment_sum(src, seg, n):
    return jax.ops.segment_sum(src, seg, n)

class _Rng:

    def __init__(self, key):
        self._k = key

    def _next(self):
        self._k, sub = jax.random.split(self._k)
        return sub

    def normal(self, shape):
        return jax.random.normal(self._next(), shape, dtype=jnp.bfloat16)

    def randint(self, lo, hi, shape):
        return jax.random.randint(self._next(), shape, lo, hi, dtype=jnp.int32)

    def uniform(self, shape, lo=0.0, hi=1.0):
        return jax.random.uniform(self._next(), shape, jnp.bfloat16, lo, hi)

    def permutation(self, n):
        return jax.random.permutation(self._next(), n)
kernel_name = 'adaLN_cond__memory_aug_recurrent_mem_tr__moe_arch_mod__prompt'

def setup_inputs():
    _rng = _Rng(jax.random.key(int.from_bytes(__import__("os").urandom(4), "little")))
    _w = lambda a: (lambda t: t.astype(jnp.bfloat16) if jnp.issubdtype(t.dtype, jnp.floating) else t)(jnp.asarray(a))

    def _A_setup():
        B, S, Dm = (1, 2048, 1024)
        H, Dh = (32, 128)
        M, seg = (8, 32)
        seg = min(seg, S)
        S = S // seg * seg
        return {'x': _w((lambda *s: _rng.normal(s) * 0.05)(B, S, Dm)), 'mem0': _w((lambda *s: _rng.normal(s) * 0.05)(B, M, Dm)), 'Wq': _w((lambda *s: _rng.normal(s) * 0.05)(Dm, H, Dh) * Dm ** (-0.5)), 'Wk': _w((lambda *s: _rng.normal(s) * 0.05)(Dm, H, Dh) * Dm ** (-0.5)), 'Wv': _w((lambda *s: _rng.normal(s) * 0.05)(Dm, H, Dh) * Dm ** (-0.5)), 'Wo': _w((lambda *s: _rng.normal(s) * 0.05)(H, Dh, Dm) * (H * Dh) ** (-0.5)), 'seg_len': seg}
    _A_in = _A_setup()

    def _B_setup():
        B, S, D, F, C = (1, 2048, 1024, 3584, 2)
        return {'x': _w((lambda *s: _rng.normal(s) * 0.05)(B, S, D)), 'w_r': _w((lambda *s: _rng.normal(s) * 0.05)(D)), 'w_gate': _w((lambda *s: _rng.normal(s) * 0.05)(D, F)), 'w_up': _w((lambda *s: _rng.normal(s) * 0.05)(D, F)), 'w_down': _w((lambda *s: _rng.normal(s) * 0.05)(F, D))}
    _B_in = _B_setup()
    return {'A_x': _A_in['x'], 'A_mem0': _A_in['mem0'], 'A_Wq': _A_in['Wq'], 'A_Wk': _A_in['Wk'], 'A_Wv': _A_in['Wv'], 'A_Wo': _A_in['Wo'], 'A_seg_len': _A_in['seg_len'], 'B_x': _B_in['x'], 'B_w_r': _B_in['w_r'], 'B_w_gate': _B_in['w_gate'], 'B_w_up': _B_in['w_up'], 'B_w_down': _B_in['w_down'], 'c': _w((lambda *s: _rng.normal(s) * 0.05)(1, 1024)), 'w_mod': _w((lambda *s: _rng.normal(s) * 0.05)(1024, 6 * 1024) * 1024 ** (-0.5))}

def reference(A_x, A_mem0, A_Wq, A_Wk, A_Wv, A_Wo, A_seg_len, B_x, B_w_r, B_w_gate, B_w_up, B_w_down, c, w_mod):

    def _A_ref(x, mem0, Wq, Wk, Wv, Wo, seg_len):
        B, S, Dm = x.shape
        H, Dh = (Wq.shape[1], Wq.shape[2])
        M = mem0.shape[1]
        scale = Dh ** (-0.5)
        n_seg = S // seg_len
        L = M + seg_len
        idx = jnp.arange(L)
        mask = (idx[:, None] < M) | (idx[:, None] >= idx[None, :])
        mem = mem0
        outs = []
        for s in range(n_seg):
            xs = x[:, s * seg_len:(s + 1) * seg_len, :].copy()
            h = jnp.concatenate([mem, xs], axis=1)
            q = jnp.einsum('btd,dhe->bhte', h, Wq)
            k = jnp.einsum('btd,dhe->bhte', h, Wk)
            v = jnp.einsum('btd,dhe->bhte', h, Wv)
            scores = jnp.einsum('bhqe,bhke->bhqk', q, k) * scale
            scores = jnp.where(mask[None, None], scores, -1000000000.0)
            p = _softmax(scores, axis=-1)
            o = jnp.einsum('bhqk,bhke->bhqe', p, v)
            o = jnp.einsum('bhte,hed->btd', o, Wo)
            mem = o[:, :M, :].copy()
            outs.append(o[:, M:, :])
        return jnp.concatenate(outs, axis=1)

    def _B_ref(x, w_r, w_gate, w_up, w_down):
        B, S, D = x.shape
        C = 2
        r = x @ w_r
        idx = jnp.argsort(-r, axis=-1)[:, :C]
        idx_e = jnp.repeat(idx.reshape(B, C, 1), D, axis=2)
        x_sel = jnp.take_along_axis(x, idx_e, axis=1)
        g = _silu(x_sel @ w_gate)
        u = x_sel @ w_up
        y = g * u @ w_down
        r_sel = _sigmoid(jnp.take_along_axis(r, idx, axis=1))
        y = y * r_sel.reshape(B, C, 1)
        b_off = (jnp.arange(B) * S).reshape(B, 1)
        flat_idx = (idx + b_off).reshape(B * C)
        zero = (x * 0.0).reshape(B * S, D)
        upd = _scatter_add(zero, flat_idx, y.reshape(B * C, D), axis=0)
        return x + upd.reshape(B, S, D)
    x = A_x
    mod = (_silu(c) @ w_mod).reshape(c.shape[0], 6, 1, -1)
    sa, ca, ga, sb, cb, gb = (mod[:, 0].copy(), mod[:, 1].copy(), mod[:, 2].copy(), mod[:, 3].copy(), mod[:, 4].copy(), mod[:, 5].copy())
    h = _layernorm(x, axis=-1) * (1 + ca) + sa
    x = x + ga * _A_ref(h, A_mem0, A_Wq, A_Wk, A_Wv, A_Wo, A_seg_len)
    h = _layernorm(x, axis=-1) * (1 + cb) + sb
    x = x + gb * _B_ref(h, B_w_r, B_w_gate, B_w_up, B_w_down)
    return x
```

```python
import functools

import jax
import jax.numpy as jnp
from jax import lax
import jax.experimental.pallas as pl
import jax.experimental.pallas.tpu as pltpu

import os
LS, LP, LW = [int(v) for v in os.environ.get('LAGS', '1,3,5').split(',')]
F32 = jnp.float32
BF16 = jnp.bfloat16
I32 = jnp.int32
EPS = 1e-5
NEG = -1000000000.0


def _rb(v):
    return v.astype(BF16).astype(F32)


def _layernorm(x):
    m = jnp.mean(x, axis=-1, keepdims=True)
    d = x - m
    v = jnp.mean(d * d, axis=-1, keepdims=True)
    return d * lax.rsqrt(v + EPS)


def _mm(a, b):
    return lax.dot_general(a, b, (((1,), (0,)), ((), ())), preferred_element_type=F32)


def _mm_nt(a, b):
    return lax.dot_general(a, b, (((1,), (1,)), ((), ())), preferred_element_type=F32)


def _build(S, D, H, E, M, SEG, FF):
    NSEG = S // SEG
    L = M + SEG
    HG = 8
    NG = H // HG
    WG = 4
    scale = float(E) ** (-0.5)

    def kernel(x_hbm, mem0_ref, wq_hbm, wk_hbm, wv_hbm, wo_hbm, wr_ref, wg_hbm, wu_hbm, wd_hbm,
               c_ref, wmod_hbm, out_hbm,
               wqkv, wo, xbuf, x1buf, outbuf, hbuf, abuf, modbuf, rbuf, wrbuf, sel, fixbuf, sems):

        def prologue(wmod_v, stq, stk, stv, sto):
            cp_mod = pltpu.make_async_copy(wmod_hbm, wmod_v, sems.at[0])
            cp_x = pltpu.make_async_copy(x_hbm, xbuf, sems.at[1])

            def wcopies(g):
                slot = g % 2
                hs = pl.ds(g * HG, HG)
                return [
                    pltpu.make_async_copy(wq_hbm.at[:, hs, :], stq.at[slot], sems.at[2 + 4 * slot]),
                    pltpu.make_async_copy(wk_hbm.at[:, hs, :], stk.at[slot], sems.at[3 + 4 * slot]),
                    pltpu.make_async_copy(wv_hbm.at[:, hs, :], stv.at[slot], sems.at[4 + 4 * slot]),
                    pltpu.make_async_copy(wo_hbm.at[pl.ds(g * HG * E, HG * E), :], sto.at[slot],
                                          sems.at[5 + 4 * slot]),
                ]

            cp_mod.start()
            cp_x.start()
            for cp in wcopies(0):
                cp.start()
            for cp in wcopies(1):
                cp.start()

            cv = c_ref[...].astype(F32)
            sc = _rb(cv * jax.nn.sigmoid(cv))
            sc8 = jnp.broadcast_to(sc, (8, D))
            cp_mod.wait()
            for j in range(6):
                mj = _rb(_mm(sc8, wmod_v[:, j * D:(j + 1) * D]))
                modbuf[j] = (1.0 + mj) if j in (1, 4) else mj
            wrbuf[...] = jnp.broadcast_to(wr_ref[...].astype(F32), (8, D))
            abuf[...] = jnp.zeros((SEG, D), F32)
            sel[...] = jnp.zeros((8, D), F32)
            hbuf[0:M, :] = mem0_ref[0].astype(F32)
            cp_x.wait()
            h0 = _rb(_layernorm(xbuf[0:SEG, :].astype(F32)) * modbuf[1, 0:1, :] + modbuf[0, 0:1, :])
            hbuf[M:L, :] = h0

            for g in range(NG):
                slot = g % 2
                cps = wcopies(g)
                for j, st in enumerate((stq, stk, stv)):
                    cps[j].wait()

                    def relayout(i, carry, st=st, j=j):
                        d0 = pl.multiple_of(i * 16, 16)
                        j0 = pl.multiple_of(i * 8, 8)
                        v = st[slot, pl.ds(d0, 16)].astype(F32)
                        v = jnp.swapaxes(v, 0, 1).astype(BF16)
                        wqkv[pl.ds(g * HG, HG), pl.ds(j0, 8), j * E:(j + 1) * E] = pltpu.bitcast(v, I32)
                        return carry

                    lax.fori_loop(0, D // 16, relayout, 0)
                cps[3].wait()

                def relayout_o(i, carry):
                    r0 = pl.multiple_of(i * 128, 128)
                    wo[pl.ds(g * HG * E // 2 + i * 64, 64), :] = pltpu.bitcast(sto[slot, pl.ds(r0, 128), :], I32)
                    return carry

                lax.fori_loop(0, HG * E // 128, relayout_o, 0)
                if g + 2 < NG:
                    for cp in wcopies(g + 2):
                        cp.start()

        pl.run_scoped(
            prologue,
            pltpu.VMEM((D, 6 * D), BF16),
            pltpu.VMEM((2, D, HG, E), BF16),
            pltpu.VMEM((2, D, HG, E), BF16),
            pltpu.VMEM((2, D, HG, E), BF16),
            pltpu.VMEM((2, HG * E, D), BF16),
        )

        def main(wg, wu, wd):
            cp_g = pltpu.make_async_copy(wg_hbm, wg, sems.at[10])
            cp_u = pltpu.make_async_copy(wu_hbm, wu, sems.at[11])
            cp_d = pltpu.make_async_copy(wd_hbm, wd, sems.at[12])
            cp_g.start()
            cp_u.start()
            cp_d.start()

            row = lax.broadcasted_iota(I32, (L, L), 0)
            col = lax.broadcasted_iota(I32, (L, L), 1)
            mask = (row < M) | (row >= col)

            def post(sp):
                xs = pl.multiple_of(jnp.maximum(sp, 0) * SEG, SEG)
                dst = pl.multiple_of((sp + 1) * SEG, SEG)
                x1 = xbuf[pl.ds(xs, SEG), :].astype(F32) + modbuf[2, 0:1, :] * abuf[...]
                h2 = _rb(_layernorm(x1) * modbuf[4, 0:1, :] + modbuf[3, 0:1, :])
                r = _rb(jnp.sum(h2 * wrbuf[0:1, :], axis=-1, keepdims=True))
                x1buf[pl.ds(dst, SEG), :] = x1
                rbuf[pl.ds(dst, SEG), :] = r
                outbuf[pl.ds(dst, SEG), :] = (x1 + modbuf[5, 0:1, :] * h2).astype(BF16)

            def step(s, carry):
                post(s - 1)
                h = hbuf[...]
                acc = None
                qkvs, ps, os_ = {}, {}, {}

                def st_qkv(hd):
                    w = pltpu.bitcast(wqkv[hd], BF16)
                    qkv = _mm(h, w)
                    qkvs[hd] = (_rb(qkv[:, 0:E]), qkv[:, E:2 * E].astype(BF16), qkv[:, 2 * E:3 * E].astype(BF16))

                def st_s(hd):
                    q, k, _ = qkvs[hd]
                    sc = _mm_nt(q, k) * scale
                    sc = jnp.where(mask, sc, NEG)
                    mx = jnp.max(sc, axis=-1, keepdims=True)
                    e = jnp.exp(sc - mx)
                    ps[hd] = (e / jnp.sum(e, axis=-1, keepdims=True)).astype(BF16)

                def st_pv(hd):
                    os_[hd] = _rb(_mm(ps[hd], qkvs[hd][2]))

                def st_wo(g, acc):
                    wog = pltpu.bitcast(wo[g * WG * E // 2:(g + 1) * WG * E // 2, :], BF16)
                    part = _mm(jnp.concatenate([os_[g * WG + j] for j in range(WG)], axis=1), wog)
                    return part if acc is None else acc + part

                for t in range(H + LW):
                    if t < H:
                        st_qkv(t)
                    if 0 <= t - LS < H:
                        st_s(t - LS)
                    if 0 <= t - LP < H:
                        st_pv(t - LP)
                    if t - LW >= 0 and (t - LW) % WG == WG - 1:
                        acc = st_wo((t - LW) // WG, acc)
                sn = pl.multiple_of(jnp.minimum(s + 1, NSEG - 1) * SEG, SEG)
                hn = _rb(_layernorm(xbuf[pl.ds(sn, SEG), :].astype(F32)) * modbuf[1, 0:1, :] + modbuf[0, 0:1, :])
                hbuf[M:L, :] = hn
                acc = _rb(acc)
                hbuf[0:M, :] = acc[0:M]
                abuf[...] = acc[M:L]
                return carry

            lax.fori_loop(0, NSEG, step, 0)
            post(NSEG - 1)

            cp_out = pltpu.make_async_copy(outbuf.at[pl.ds(SEG, S), :], out_hbm, sems.at[13])
            cp_out.start()

            r_all = rbuf[pl.ds(SEG, S), :]
            idx = lax.broadcasted_iota(I32, (S, 1), 0)
            m1 = jnp.max(r_all)
            i1 = jnp.min(jnp.where(r_all == m1, idx, S))
            r_rest = jnp.where(idx == i1, -jnp.inf, r_all)
            m2 = jnp.max(r_rest)
            i2 = jnp.min(jnp.where((r_rest == m2) & (idx != i1), idx, S))
            i1 = jnp.clip(i1, 0, S - 1)
            i2 = jnp.clip(i2, 0, S - 1)

            x1a = x1buf[pl.ds(i1 + SEG, 1), :]
            x1b = x1buf[pl.ds(i2 + SEG, 1), :]
            h2a = _rb(_layernorm(x1a) * modbuf[4, 0:1, :] + modbuf[3, 0:1, :])
            h2b = _rb(_layernorm(x1b) * modbuf[4, 0:1, :] + modbuf[3, 0:1, :])
            sel[0:1, :] = h2a
            sel[1:2, :] = h2b
            xs = sel[...]
            cp_g.wait()
            cp_u.wait()
            gq = _rb(_mm(xs, wg[...]))
            uq = _rb(_mm(xs, wu[...]))
            act = _rb(_rb(gq * jax.nn.sigmoid(gq)) * uq)
            cp_d.wait()
            y = _rb(_mm(act, wd[...]))
            sig1 = _rb(jax.nn.sigmoid(jnp.full((1, D), m1, F32)))
            sig2 = _rb(jax.nn.sigmoid(jnp.full((1, D), m2, F32)))
            row1 = x1a + modbuf[5, 0:1, :] * (h2a + _rb(y[0:1] * sig1))
            row2 = x1b + modbuf[5, 0:1, :] * (h2b + _rb(y[1:2] * sig2))

            bases = []
            for n, ii in enumerate((i1, i2)):
                b = pl.multiple_of((ii // 16) * 16, 16)
                gidx = b + lax.broadcasted_iota(I32, (16, D), 0)
                blk = outbuf[pl.ds(b + SEG, 16), :].astype(F32)
                blk = jnp.where(gidx == i1, row1, jnp.where(gidx == i2, row2, blk))
                fixbuf[n] = blk.astype(BF16)
                bases.append(b)
            cp_out.wait()
            for n, b in enumerate(bases):
                cp = pltpu.make_async_copy(fixbuf.at[n], out_hbm.at[pl.ds(b, 16), :], sems.at[14])
                cp.start()
                cp.wait()

        pl.run_scoped(
            main,
            pltpu.VMEM((D, FF), BF16),
            pltpu.VMEM((D, FF), BF16),
            pltpu.VMEM((FF, D), BF16),
        )

    any_spec = pl.BlockSpec(memory_space=pl.ANY)
    vmem_spec = pl.BlockSpec(memory_space=pltpu.VMEM)
    return pl.pallas_call(
        kernel,
        out_shape=jax.ShapeDtypeStruct((S, D), BF16),
        in_specs=[any_spec, vmem_spec, any_spec, any_spec, any_spec, any_spec, vmem_spec,
                  any_spec, any_spec, any_spec, vmem_spec, any_spec],
        out_specs=any_spec,
        scratch_shapes=[
            pltpu.VMEM((H, D // 2, 3 * E), I32),
            pltpu.VMEM((H * E // 2, D), I32),
            pltpu.VMEM((S, D), BF16),
            pltpu.VMEM((S + SEG, D), F32),
            pltpu.VMEM((S + SEG, D), BF16),
            pltpu.VMEM((L, D), F32),
            pltpu.VMEM((SEG, D), F32),
            pltpu.VMEM((6, 8, D), F32),
            pltpu.VMEM((S + SEG, 1), F32),
            pltpu.VMEM((8, D), F32),
            pltpu.VMEM((8, D), F32),
            pltpu.VMEM((2, 16, D), BF16),
            pltpu.SemaphoreType.DMA((16,)),
        ],
        compiler_params=pltpu.CompilerParams(vmem_limit_bytes=120 * 1024 * 1024),
        name="adaln_rmt_mod",
    )


@functools.partial(jax.jit, static_argnames=("A_seg_len",))
def pallas_adaLN_cond__memory_aug_recurrent_mem_tr__moe_arch_mod__prompt_kernel(
    A_x: jax.Array,
    A_mem0: jax.Array,
    A_Wq: jax.Array,
    A_Wk: jax.Array,
    A_Wv: jax.Array,
    A_Wo: jax.Array,
    A_seg_len: int,
    B_x: jax.Array,
    B_w_r: jax.Array,
    B_w_gate: jax.Array,
    B_w_up: jax.Array,
    B_w_down: jax.Array,
    c: jax.Array,
    w_mod: jax.Array,
):
    del B_x
    B, S, D = A_x.shape
    H, E = A_Wq.shape[1], A_Wq.shape[2]
    M = A_mem0.shape[1]
    SEG = int(A_seg_len)
    FF = B_w_gate.shape[1]
    assert B == 1 and S % SEG == 0
    call = _build(S, D, H, E, M, SEG, FF)
    out = call(
        A_x.reshape(S, D), A_mem0, A_Wq, A_Wk, A_Wv, A_Wo.reshape(H * E, D),
        B_w_r.reshape(1, D), B_w_gate, B_w_up, B_w_down, c, w_mod,
    )
    return out.reshape(B, S, D)
```

```python
import functools

import jax
import jax.numpy as jnp
from jax import lax
import jax.experimental.pallas as pl
import jax.experimental.pallas.tpu as pltpu

import os
LS, LP, LW = [int(v) for v in os.environ.get('LAGS', '1,3,5').split(',')]
F32 = jnp.float32
BF16 = jnp.bfloat16
I32 = jnp.int32
EPS = 1e-5
NEG = -1000000000.0
LOG2E = 1.4426950408889634


def _rb(v):
    return v.astype(BF16).astype(F32)


def _layernorm(x):
    m = jnp.mean(x, axis=-1, keepdims=True)
    d = x - m
    v = jnp.mean(d * d, axis=-1, keepdims=True)
    return d * lax.rsqrt(v + EPS)


def _mm(a, b):
    return lax.dot_general(a, b, (((1,), (0,)), ((), ())), preferred_element_type=F32)


def _mm_nt(a, b):
    return lax.dot_general(a, b, (((1,), (1,)), ((), ())), preferred_element_type=F32)


def _transpose4(v):
    sub = lax.broadcasted_iota(I32, (8, 128), 0)
    v = list(v)
    for k in (2, 1):
        m = (sub & k) != 0
        for i in range(4):
            if i & k:
                continue
            a, b = v[i], v[i + k]
            v[i] = jnp.where(m, pltpu.roll(b, k, 0), a)
            v[i + k] = jnp.where(m, b, pltpu.roll(a, 8 - k, 0))
    return v


def _build(S, D, H, E, M, SEG, FF):
    NSEG = S // SEG
    L = M + SEG
    HG = 8
    NG = H // HG
    WG = 4
    scale = float(E) ** (-0.5)

    NRUN = int(os.environ.get('NSTEPS', NSEG))
    LT = 24
    NL = int(os.environ.get('NL', 24))
    T = NL * (SEG - LT)
    R = 288
    assert T % LT == 0 and R % LT == 0 and R % SEG == 0 and R >= T + LT and T % 16 == 0
    XA = -(-(T + 3 * LT) // 16) * 16
    ND = D // 128
    NF = FF // 128
    WOG = [int(v) for v in os.environ.get('WOG', '4,4,4,4,4,4,4,3,1').split(',')] if H == 32 else [H]
    SCHED = []
    ends = {}
    h0 = 0
    for n in WOG:
        ends[h0 + n - 1] = (h0, n)
        h0 += n
    for t in range(H + LW):
        if t < H:
            SCHED.append(("q", t))
        if 0 <= t - LS < H:
            SCHED.append(("s", t - LS))
        if 0 <= t - LP < H:
            SCHED.append(("p", t - LP))
        if t - LW in ends:
            SCHED.append(("w", ends[t - LW]))
    if os.environ.get("TAIL") and H == 32:
        cut = SCHED.index(("q", 31)) + 1
        head = [e for e in SCHED[:cut]]
        tail = []
        for tok in os.environ["TAIL"].split():
            if tok[0] in "ps":
                tail.append((tok[0], int(tok[1:])))
            else:
                a, b = tok[1:].split(":")
                tail.append(("w", (int(a), int(b))))
        done = {e for e in head}
        head = [e for e in head if e not in tail]
        SCHED = head + tail
    REST_STEP = 2
    PL = 2

    def kernel(x_hbm, mem0_ref, wq_hbm, wk_hbm, wv_hbm, wo_hbm, wr_ref, wg_hbm, wu_hbm, wd_hbm,
               c_ref, wmod_hbm, out_hbm,
               wqkv, wo, wmod, wg, wu, wd, stq, stk, stv,
               xbuf, abuf, outbuf, hbuf, modbuf, wrbuf, sel, fixbuf, ring, hT, sems):

        def slab_copies(src, dst, js, sem):
            return [pltpu.make_async_copy(src.at[:, pl.ds(j * 128, 128)], dst.at[j].bitcast(BF16), sem)
                    for j in js]

        def start(cps):
            for cp in cps:
                cp.start()

        def wait(cps):
            for cp in cps:
                cp.wait()

        cp_mod0 = slab_copies(wmod_hbm, wmod, range(0, 2 * ND), sems.at[0])
        cp_mod1 = slab_copies(wmod_hbm, wmod, range(2 * ND, 6 * ND), sems.at[1])
        cp_xa = [pltpu.make_async_copy(x_hbm.at[pl.ds(0, XA), :], xbuf.at[pl.ds(0, XA), :], sems.at[2])]
        cp_xb = [pltpu.make_async_copy(x_hbm.at[pl.ds(XA, S - XA), :], xbuf.at[pl.ds(XA, S - XA), :], sems.at[3])]
        cp_wo = slab_copies(wo_hbm, wo, range(ND), sems.at[4])
        cp_ffn = (slab_copies(wg_hbm, wg, range(NF), sems.at[5]) + slab_copies(wu_hbm, wu, range(NF), sems.at[5])
                  + slab_copies(wd_hbm, wd, range(ND), sems.at[5]))

        def wcopies(g):
            slot = g % 2
            hs = pl.ds(g * HG, HG)
            return [pltpu.make_async_copy(w.at[:, hs, :], st.at[slot], sems.at[6 + 3 * slot + j])
                    for j, (w, st) in enumerate(((wq_hbm, stq), (wk_hbm, stk), (wv_hbm, stv)))]

        def mod_vectors(js):
            cv = c_ref[...].astype(F32)
            sc8 = jnp.broadcast_to(_rb(cv * jax.nn.sigmoid(cv)), (8, D))
            for j in js:
                mj = jnp.concatenate(
                    [_mm(sc8, pltpu.bitcast(wmod[j * ND + n], BF16)) for n in range(ND)], axis=1)
                mj = _rb(mj)
                modbuf[j] = (1.0 + mj) if j in (1, 4) else mj

        def pre(xs):
            return _rb(_layernorm(xs.astype(F32)) * modbuf[1, 0:1, :] + modbuf[0, 0:1, :])

        start(cp_mod0)
        start(cp_xa)
        start(wcopies(0))
        start(wcopies(1))
        wrbuf[...] = jnp.broadcast_to(wr_ref[...].astype(F32).reshape(1, D), (8, D))
        sel[...] = jnp.zeros((8, D), F32)
        hbuf[0:M, :] = mem0_ref[0].astype(F32)
        wait(cp_mod0)
        mod_vectors((0, 1))
        wait(cp_xa)

        def pre_loop(i, carry):
            r0 = pl.multiple_of(i * 16, 16)
            hT[pl.ds(r0, 16), :] = pre(xbuf[pl.ds(r0, 16), :]).astype(BF16)
            return carry

        lax.fori_loop(0, T // 16, pre_loop, 0)
        hbuf[M:M + LT, :] = pre(xbuf[T:T + LT, :])

        for g in range(NG):
            slot = g % 2
            cps = wcopies(g)
            for j, st in enumerate((stq, stk, stv)):
                cps[j].wait()
                if g == NG - 1 and j == 0:
                    start(cp_wo)
                if g == NG - 1 and j == 2:
                    start(cp_mod1)
                    start(cp_xb)

                def relayout(i, carry, st=st, j=j):
                    for u in range(2):
                        d0 = pl.multiple_of(i * 32 + u * 16, 16)
                        j0 = pl.multiple_of(i * 16 + u * 8, 8)
                        blk = st[slot, pl.ds(d0, 16)]
                        ev, od = [
                            _transpose4([pltpu.bitcast(jnp.concatenate([blk[2 * a + p], blk[2 * a + p + 8]], axis=0), I32)
                                         for a in range(4)]) for p in (0, 1)]
                        for hp in range(HG // 2):
                            lo = (ev[hp] & 0xFFFF) | (od[hp] << 16)
                            hi = lax.shift_right_logical(ev[hp], 16) | (od[hp] & jnp.int32(-65536))
                            wqkv[g * HG + 2 * hp, pl.ds(j0, 8), j * E:(j + 1) * E] = lo
                            wqkv[g * HG + 2 * hp + 1, pl.ds(j0, 8), j * E:(j + 1) * E] = hi
                    return carry

                lax.fori_loop(0, D // 32, relayout, 0)
            if g + 2 < NG:
                start(wcopies(g + 2))

            def project(i, carry, g=g):
                for u in range(2):
                    hd = g * HG + i * 2 + u
                    ring[hd, 0:T, :] = _mm(hT[...], pltpu.bitcast(wqkv[hd], BF16))
                return carry

            lax.fori_loop(0, HG // 2, project, 0)
        wait(cp_wo)

        row = lax.broadcasted_iota(I32, (L, L), 0)
        col = lax.broadcasted_iota(I32, (L, L), 1)
        mask = (row < M) | (row >= col)

        def second_half():
            wait(cp_mod1)
            wait(cp_xb)
            start(cp_ffn)
            mod_vectors((2, 3, 4, 5))

        def residual(xs, a):
            x1 = xs.astype(F32) + modbuf[2, 0:1, :] * a.astype(F32)
            h2 = _rb(_layernorm(x1) * modbuf[4, 0:1, :] + modbuf[3, 0:1, :])
            return x1, h2

        def out_copy(sp):
            dst = pl.multiple_of(jnp.maximum(sp, 0) * SEG, SEG)
            src = pl.multiple_of((sp + PL) * SEG, SEG)
            return pltpu.make_async_copy(outbuf.at[pl.ds(src, SEG), :], out_hbm.at[pl.ds(dst, SEG), :], sems.at[12])

        def post(sp, top):
            src = pl.multiple_of(jnp.maximum(sp, 0) * SEG, SEG)
            dst = pl.multiple_of((sp + PL) * SEG, SEG)
            a = jnp.where(sp >= 0, abuf[pl.ds(src, SEG), :].astype(F32), 0.0)
            x1, h2 = residual(xbuf[pl.ds(src, SEG), :], a)
            outbuf[pl.ds(dst, SEG), :] = (x1 + modbuf[5, 0:1, :] * h2).astype(BF16)
            r = _rb(jnp.sum(h2 * wrbuf[0:1, :], axis=-1, keepdims=True))
            r = jnp.where(sp >= 0, r, -jnp.inf)
            b1, i1, b2, i2 = top
            sub = lax.broadcasted_iota(I32, (8, 1), 0)
            for t in range(SEG // 8):
                rv = r[t * 8:(t + 1) * 8]
                iv = src + t * 8 + sub
                g1 = rv > b1
                g2 = rv > b2
                b2 = jnp.where(g1, b1, jnp.where(g2, rv, b2))
                i2 = jnp.where(g1, i1, jnp.where(g2, iv, i2))
                b1 = jnp.where(g1, rv, b1)
                i1 = jnp.where(g1, iv, i1)
            return b1, i1, b2, i2

        def step(s, top, light):
            if light:
                pl.when(s == REST_STEP)(second_half)
            top = post(s - PL, top)
            nt = LT if light else SEG
            h = hbuf[0:M + nt, :]
            acc = None
            qkvs, ps, os_ = {}, {}, {}
            if light:
                ppos = pl.multiple_of(lax.rem(T + s * LT, R), 8)
                apos = pl.multiple_of(lax.rem(s * SEG, R), SEG)

            def st_qkv(hd):
                w = pltpu.bitcast(wqkv[hd], BF16)
                qkv = lax.dot_general(h, w, (((1,), (0,)), ((), ())), preferred_element_type=F32)
                if light:
                    ring[hd, pl.ds(ppos, LT), :] = qkv[M:]
                    qkvs[hd] = qkv[0:M]
                else:
                    qkvs[hd] = qkv

            pref = {}

            def prefetch(i):
                for kind, a in SCHED[i + 1:]:
                    if kind == "q":
                        break
                    for j in {"s": (0, 1), "p": (2,), "w": ()}[kind]:
                        pref[a, j] = ring[a, pl.ds(apos, SEG), j * E:(j + 1) * E]

            def part(hd, j):
                v = qkvs[hd][:, j * E:(j + 1) * E]
                if light:
                    v = jnp.concatenate([v, pref[hd, j]], axis=0)
                return v

            def st_s(hd):
                q = _rb(part(hd, 0))
                k = part(hd, 1).astype(BF16)
                sc = lax.dot_general(q, k, (((1,), (1,)), ((), ())), preferred_element_type=F32)
                sc = jnp.where(mask, sc, NEG / scale)
                mx = jnp.max(sc, axis=-1, keepdims=True)
                e = jnp.exp2((sc - mx) * (scale * LOG2E))
                ps[hd] = (_rb(e), 1.0 / jnp.sum(e, axis=-1, keepdims=True))

            def st_pv(hd):
                e, inv = ps[hd]
                v = part(hd, 2).astype(BF16)
                pv = lax.dot_general(e, v, (((1,), (0,)), ((), ())), preferred_element_type=F32)
                os_[hd] = _rb(pv * inv)

            def st_wo(h0, n, acc):
                o = jnp.concatenate([os_[h0 + j] for j in range(n)], axis=1)
                part = jnp.concatenate(
                    [_mm(o, pltpu.bitcast(wo[j, h0 * E // 2:(h0 + n) * E // 2, :], BF16)) for j in range(ND)], axis=1)
                return part if acc is None else acc + part

            for i, (kind, a) in enumerate(SCHED):
                if kind == "q":
                    if light:
                        prefetch(i)
                    st_qkv(a)
                elif kind == "s":
                    st_s(a)
                elif kind == "p":
                    st_pv(a)
                else:
                    acc = st_wo(a[0], a[1], acc)
            if light:
                sn = pl.multiple_of(T + jnp.minimum(s + 1, NL - 1) * LT, 8)
            else:
                sn = pl.multiple_of(jnp.minimum(s + 1, NSEG - 1) * SEG, SEG)
            hbuf[M:M + nt, :] = pre(xbuf[pl.ds(sn, nt), :])
            acc = _rb(acc)
            hbuf[0:M, :] = acc[0:M]
            abuf[pl.ds(pl.multiple_of(s * SEG, SEG), SEG), :] = acc[M:L].astype(BF16)

            @pl.when(s >= PL)
            def _():
                out_copy(s - PL).start()
            return top

        ninf = jnp.full((8, 1), -jnp.inf, F32)
        izero = jnp.zeros((8, 1), I32)
        top = lax.fori_loop(0, NL, functools.partial(step, light=True), (ninf, izero, ninf, izero))
        hbuf[M:L, :] = pre(xbuf[NL * SEG:(NL + 1) * SEG, :])
        top = lax.fori_loop(NL, NRUN, functools.partial(step, light=False), top)
        for sp in range(NSEG - PL, NSEG):
            top = post(sp, top)
            out_copy(sp).start()

        b1, i1v, b2, i2v = top
        m1 = jnp.max(b1)
        i1 = jnp.min(jnp.where(b1 == m1, i1v, S))
        win = (b1 == m1) & (i1v == i1)
        c1 = jnp.where(win, b2, b1)
        ci = jnp.where(win, i2v, i1v)
        m2 = jnp.max(c1)
        i2 = jnp.min(jnp.where(c1 == m2, ci, S))
        i1 = jnp.clip(i1, 0, S - 1)
        i2 = jnp.clip(i2, 0, S - 1)

        rows = []
        for n, ii in enumerate((i1, i2)):
            b = pl.multiple_of((ii // 16) * 16, 16)
            gidx = b + lax.broadcasted_iota(I32, (16, D), 0)
            x1, h2 = residual(xbuf[pl.ds(b, 16), :], abuf[pl.ds(b, 16), :])
            hit = gidx == ii
            x1 = jnp.sum(jnp.where(hit, x1, 0.0), axis=0, keepdims=True)
            h2 = jnp.sum(jnp.where(hit, h2, 0.0), axis=0, keepdims=True)
            sel[n:n + 1, :] = h2
            rows.append((b, x1, h2))
        xs = sel[...]
        wait(cp_ffn)
        acts = []
        for j in range(NF):
            gq = _rb(_mm(xs, pltpu.bitcast(wg[j], BF16)))
            uq = _rb(_mm(xs, pltpu.bitcast(wu[j], BF16)))
            acts.append(_rb(_rb(gq * jax.nn.sigmoid(gq)) * uq))
        act = jnp.concatenate(acts, axis=1)
        y = _rb(jnp.concatenate([_mm(act, pltpu.bitcast(wd[j], BF16)) for j in range(ND)], axis=1))
        new = []
        for n, mm in enumerate((m1, m2)):
            _, x1, h2 = rows[n]
            sig = _rb(jax.nn.sigmoid(jnp.full((1, D), mm, F32)))
            new.append(x1 + modbuf[5, 0:1, :] * (h2 + _rb(y[n:n + 1] * sig)))
        for n in range(2):
            b = rows[n][0]
            gidx = b + lax.broadcasted_iota(I32, (16, D), 0)
            blk = outbuf[pl.ds(b + PL * SEG, 16), :].astype(F32)
            blk = jnp.where(gidx == i1, new[0], jnp.where(gidx == i2, new[1], blk))
            fixbuf[n] = blk.astype(BF16)
        pltpu.make_async_copy(outbuf.at[pl.ds(PL * SEG, NRUN * SEG), :], out_hbm.at[pl.ds(0, NRUN * SEG), :], sems.at[12]).wait()
        for n in range(2):
            cp = pltpu.make_async_copy(fixbuf.at[n], out_hbm.at[pl.ds(rows[n][0], 16), :], sems.at[13])
            cp.start()
            cp.wait()

    any_spec = pl.BlockSpec(memory_space=pl.ANY)
    vmem_spec = pl.BlockSpec(memory_space=pltpu.VMEM)
    return pl.pallas_call(
        kernel,
        out_shape=jax.ShapeDtypeStruct((S, D), BF16),
        in_specs=[any_spec, vmem_spec, any_spec, any_spec, any_spec, any_spec, vmem_spec,
                  any_spec, any_spec, any_spec, vmem_spec, any_spec],
        out_specs=any_spec,
        scratch_shapes=[
            pltpu.VMEM((H, D // 2, 3 * E), I32),
            pltpu.VMEM((ND, H * E // 2, 128), I32),
            pltpu.VMEM((6 * ND, D // 2, 128), I32),
            pltpu.VMEM((NF, D // 2, 128), I32),
            pltpu.VMEM((NF, D // 2, 128), I32),
            pltpu.VMEM((ND, FF // 2, 128), I32),
            pltpu.VMEM((2, D, HG, E), BF16),
            pltpu.VMEM((2, D, HG, E), BF16),
            pltpu.VMEM((2, D, HG, E), BF16),
            pltpu.VMEM((S, D), BF16),
            pltpu.VMEM((S, D), BF16),
            pltpu.VMEM((S + PL * SEG, D), BF16),
            pltpu.VMEM((L, D), F32),
            pltpu.VMEM((6, 8, D), F32),
            pltpu.VMEM((8, D), F32),
            pltpu.VMEM((8, D), F32),
            pltpu.VMEM((2, 16, D), BF16),
            pltpu.VMEM((H, R, 3 * E), F32),
            pltpu.VMEM((T, D), BF16),
            pltpu.SemaphoreType.DMA((16,)),
        ],
        compiler_params=pltpu.CompilerParams(vmem_limit_bytes=120 * 1024 * 1024),
        name="adaln_rmt_mod",
    )


@functools.partial(jax.jit, static_argnames=("A_seg_len",))
def pallas_adaLN_cond__memory_aug_recurrent_mem_tr__moe_arch_mod__prompt_kernel(
    A_x: jax.Array,
    A_mem0: jax.Array,
    A_Wq: jax.Array,
    A_Wk: jax.Array,
    A_Wv: jax.Array,
    A_Wo: jax.Array,
    A_seg_len: int,
    B_x: jax.Array,
    B_w_r: jax.Array,
    B_w_gate: jax.Array,
    B_w_up: jax.Array,
    B_w_down: jax.Array,
    c: jax.Array,
    w_mod: jax.Array,
):
    del B_x
    B, S, D = A_x.shape
    H, E = A_Wq.shape[1], A_Wq.shape[2]
    M = A_mem0.shape[1]
    SEG = int(A_seg_len)
    FF = B_w_gate.shape[1]
    assert B == 1 and S % SEG == 0
    call = _build(S, D, H, E, M, SEG, FF)
    out = call(
        A_x.reshape(S, D), A_mem0, A_Wq, A_Wk, A_Wv, A_Wo.reshape(H * E, D),
        B_w_r, B_w_gate, B_w_up, B_w_down, c, w_mod,
    )
    return out.reshape(B, S, D)
```

```python
import functools

import jax
import jax.numpy as jnp
from jax import lax
import jax.experimental.pallas as pl
import jax.experimental.pallas.tpu as pltpu

import os
LS, LP, LW = [int(v) for v in os.environ.get('LAGS', '1,3,5').split(',')]
F32 = jnp.float32
import contextlib
_sc = (lambda n: jax.named_scope(n)) if os.environ.get('PROF') else (lambda n: contextlib.nullcontext())
BF16 = jnp.bfloat16
I32 = jnp.int32
EPS = 1e-5
NEG = -1000000000.0
LOG2E = 1.4426950408889634


def _rb(v):
    return v.astype(BF16).astype(F32)


def _layernorm(x):
    m = jnp.mean(x, axis=-1, keepdims=True)
    d = x - m
    v = jnp.mean(d * d, axis=-1, keepdims=True)
    return d * lax.rsqrt(v + EPS)


def _mm(a, b):
    return lax.dot_general(a, b, (((1,), (0,)), ((), ())), preferred_element_type=F32)


def _mm_nt(a, b):
    return lax.dot_general(a, b, (((1,), (1,)), ((), ())), preferred_element_type=F32)


def _transpose4(v):
    sub = lax.broadcasted_iota(I32, (8, 128), 0)
    v = list(v)
    for k in (2, 1):
        m = (sub & k) != 0
        for i in range(4):
            if i & k:
                continue
            a, b = v[i], v[i + k]
            v[i] = jnp.where(m, pltpu.roll(b, k, 0), a)
            v[i + k] = jnp.where(m, b, pltpu.roll(a, 8 - k, 0))
    return v


def _build(S, D, H, E, M, SEG, FF):
    NSEG = S // SEG
    L = M + SEG
    HG = 8
    NG = H // HG
    WG = 4
    scale = float(E) ** (-0.5)

    NRUN = int(os.environ.get('NSTEPS', NSEG))
    LT = 24
    NL = int(os.environ.get('NL', 30))
    T = NL * (SEG - LT)
    R = 288
    assert T % LT == 0 and R % LT == 0 and R % SEG == 0 and R >= T + LT and T % 16 == 0
    XA = -(-(T + 3 * LT) // 16) * 16
    ND = D // 128
    NF = FF // 128
    WOG = [int(v) for v in os.environ.get('WOG', '4,4,4,4,4,4,4,3,1').split(',')] if H == 32 else [H]
    SCHED = []
    ends = {}
    h0 = 0
    for n in WOG:
        ends[h0 + n - 1] = (h0, n)
        h0 += n
    for t in range(H + LW):
        if t < H:
            SCHED.append(("q", t))
        if 0 <= t - LS < H:
            SCHED.append(("s", t - LS))
        if 0 <= t - LP < H:
            SCHED.append(("p", t - LP))
        if t - LW in ends:
            SCHED.append(("w", ends[t - LW]))
    if H == 32:
        cut = SCHED.index(("q", 31)) + 1
        head = [e for e in SCHED[:cut]]
        tail = []
        for tok in os.environ.get("TAIL", "s30 p28 p29 w24:1 s31 w25:2 p30 w27:1 p31 w28:2 w30:1 w31:1").split():
            if tok[0] in "ps":
                tail.append((tok[0], int(tok[1:])))
            else:
                a, b = tok[1:].split(":")
                tail.append(("w", (int(a), int(b))))
        done = {e for e in head}
        head = [e for e in head if e not in tail]
        SCHED = head + tail
    A_POST, A_PRE, A_D = [int(v) for v in os.environ.get('ANCH', '2,0,4').split(',')]
    REST_STEP = 2
    PL = 2

    def kernel(x_hbm, mem0_ref, wq_hbm, wk_hbm, wv_hbm, wo_hbm, wr_ref, wg_hbm, wu_hbm, wd_hbm,
               c_ref, wmod_hbm, out_hbm,
               wqkv, wo, wmod, wg, wu, wd, stg,
               xbuf, abuf, outbuf, hbuf, modbuf, wrbuf, sel, fixbuf, ring, hT, zs, sems):

        def slab_copies(src, dst, js, sem):
            return [pltpu.make_async_copy(src.at[:, pl.ds(j * 128, 128)], dst.at[j].bitcast(BF16), sem)
                    for j in js]

        def start(cps):
            for cp in cps:
                cp.start()

        def wait(cps):
            for cp in cps:
                cp.wait()

        cp_mod0 = slab_copies(wmod_hbm, wmod, range(0, 2 * ND), sems.at[0])
        cp_mod1 = slab_copies(wmod_hbm, wmod, range(2 * ND, 6 * ND), sems.at[1])
        cp_xa = [pltpu.make_async_copy(x_hbm.at[pl.ds(0, XA), :], xbuf.at[pl.ds(0, XA), :], sems.at[2])]
        cp_xb = [pltpu.make_async_copy(x_hbm.at[pl.ds(XA, S - XA), :], xbuf.at[pl.ds(XA, S - XA), :], sems.at[3])]
        cp_wo = slab_copies(wo_hbm, wo, range(ND), sems.at[4])
        cp_ffn = (slab_copies(wg_hbm, wg, range(NF), sems.at[5]) + slab_copies(wu_hbm, wu, range(NF), sems.at[5])
                  + slab_copies(wd_hbm, wd, range(ND), sems.at[5]))

        def wcopies(g):
            slot = g % 2
            hs = pl.ds(pl.multiple_of(g * HG, HG), HG)
            return [pltpu.make_async_copy(w.at[:, hs, :], stg.at[slot, j], sems.at[6 + 3 * slot + j])
                    for j, w in enumerate((wq_hbm, wk_hbm, wv_hbm))]

        def mod_vectors(js):
            cv = c_ref[...].astype(F32)
            sc8 = jnp.broadcast_to(_rb(cv * jax.nn.sigmoid(cv)), (8, D))
            for j in js:
                mj = jnp.concatenate(
                    [_mm(sc8, pltpu.bitcast(wmod[j * ND + n], BF16)) for n in range(ND)], axis=1)
                mj = _rb(mj)
                modbuf[j] = (1.0 + mj) if j in (1, 4) else mj

        def pre(xs):
            return _rb(_layernorm(xs.astype(F32)) * modbuf[1, 0:1, :] + modbuf[0, 0:1, :])

        zs[0] = 0
        start(cp_mod0)
        start(cp_xa)
        start(wcopies(0))
        start(wcopies(1))
        wrbuf[...] = jnp.broadcast_to(wr_ref[...].astype(F32).reshape(1, D), (8, D))
        sel[...] = jnp.zeros((8, D), F32)
        hbuf[0:M, :] = mem0_ref[0].astype(F32)
        with _sc("p0_waitmod"):
            wait(cp_mod0)
        mod_vectors((0, 1))
        wait(cp_xa)

        def pre_loop(i, carry):
            r0 = pl.multiple_of(i * 48, 16)
            hT[pl.ds(r0, 48), :] = pre(xbuf[pl.ds(r0, 48), :]).astype(BF16)
            return carry

        lax.fori_loop(0, T // 48, pre_loop, 0)
        hbuf[M:M + LT, :] = pre(xbuf[T:T + LT, :])

        def relayout(g, j, d0):
            d0 = pl.multiple_of(d0, 16)
            blk = stg[g % 2, j, pl.ds(d0, 16)]
            ev, od = [
                _transpose4([pltpu.bitcast(jnp.concatenate([blk[2 * a + p], blk[2 * a + p + 8]], axis=0), I32)
                             for a in range(4)]) for p in (0, 1)]
            rows = pl.ds(pl.multiple_of(d0 // 2, 8), 8)
            cols = pl.ds(pl.multiple_of(j * E, E), E)
            for hp in range(HG // 2):
                wqkv[g * HG + 2 * hp, rows, cols] = (ev[hp] & 0xFFFF) | (od[hp] << 16)
                wqkv[g * HG + 2 * hp + 1, rows, cols] = (
                    lax.shift_right_logical(ev[hp], 16) | (od[hp] & jnp.int32(-65536)))

        def project(hd):
            ring[hd, 0:T, :] = _mm(hT[...], pltpu.bitcast(wqkv[hd], BF16))

        def project_pair(i, carry):
            project(2 * i)
            project(2 * i + 1)
            return carry

        cp0 = wcopies(0)
        with _sc("p1_first"):
            for j in range(3):
                cp0[j].wait()

                def rl(i, carry, j=j):
                    relayout(0, j, i * 32)
                    relayout(0, j, i * 32 + 16)
                    return carry

                lax.fori_loop(0, D // 32, rl, 0)
        start(wcopies(2))

        def group(g, carry):
            project_pair(g * (HG // 2), 0)

            def fused(j, carry):
                pltpu.make_async_copy(wq_hbm.at[:, pl.ds(0, HG), :], stg.at[(g + 1) % 2, j],
                                      sems.at[6 + 3 * ((g + 1) % 2) + j]).wait()

                def inner(u, carry):
                    project(g * HG + 2 + 2 * j + u)
                    for w in range(D // 32):
                        relayout(g + 1, j, u * (D // 2) + w * 16)
                    return carry

                return lax.fori_loop(0, 2, inner, carry)

            lax.fori_loop(0, 3, fused, 0)

            @pl.when(g == 0)
            def _():
                start(wcopies(3))
                start(cp_wo)
                start(cp_mod1)
                start(cp_xb)
            return carry

        assert NG == 4 and HG == 8
        with _sc("p3_project"):
            lax.fori_loop(0, NG - 1, group, 0)
            lax.fori_loop(H // 2 - HG // 2, H // 2, project_pair, 0)
        with _sc("p4_waitwo"):
            wait(cp_wo)

        row = lax.broadcasted_iota(I32, (L, L), 0)
        col = lax.broadcasted_iota(I32, (L, L), 1)
        mask = (row < M) | (row >= col)

        def second_half():
            wait(cp_mod1)
            wait(cp_xb)
            start(cp_ffn)
            mod_vectors((2, 3, 4, 5))

        def residual(xs, a):
            x1 = xs.astype(F32) + modbuf[2, 0:1, :] * a.astype(F32)
            h2 = _rb(_layernorm(x1) * modbuf[4, 0:1, :] + modbuf[3, 0:1, :])
            return x1, h2

        def out_copy(sp):
            dst = pl.multiple_of(jnp.maximum(sp, 0) * SEG, SEG)
            src = pl.multiple_of((sp + PL) * SEG, SEG)
            return pltpu.make_async_copy(outbuf.at[pl.ds(src, SEG), :], out_hbm.at[pl.ds(dst, SEG), :], sems.at[12])

        def post(sp, top):
            src = pl.multiple_of(jnp.maximum(sp, 0) * SEG, SEG)
            dst = pl.multiple_of((sp + PL) * SEG, SEG)
            a = jnp.where(sp >= 0, abuf[pl.ds(src, SEG), :].astype(F32), 0.0)
            x1, h2 = residual(xbuf[pl.ds(src, SEG), :], a)
            outbuf[pl.ds(dst, SEG), :] = (x1 + modbuf[5, 0:1, :] * h2).astype(BF16)
            r = _rb(jnp.sum(h2 * wrbuf[0:1, :], axis=-1, keepdims=True))
            r = jnp.where(sp >= 0, r, -jnp.inf)
            b1, i1, b2, i2 = top
            sub = lax.broadcasted_iota(I32, (8, 1), 0)
            for t in range(SEG // 8):
                rv = r[t * 8:(t + 1) * 8]
                iv = src + t * 8 + sub
                g1 = rv > b1
                g2 = rv > b2
                b2 = jnp.where(g1, b1, jnp.where(g2, rv, b2))
                i2 = jnp.where(g1, i1, jnp.where(g2, iv, i2))
                b1 = jnp.where(g1, rv, b1)
                i1 = jnp.where(g1, iv, i1)
            return b1, i1, b2, i2

        def step(s, top, light):
            if light:
                pl.when(s == REST_STEP)(second_half)
            nt = LT if light else SEG
            anchor = H + zs[0]
            h = hbuf[0:M + nt, :]
            acc = None
            qkvs, ps, os_ = {}, {}, {}
            if light:
                ppos = pl.multiple_of(lax.rem(T + s * LT, R), 8)
                apos = pl.multiple_of(lax.rem(s * SEG, R), SEG)

            def st_qkv(hd):
                w = pltpu.bitcast(wqkv[hd], BF16)
                qkv = lax.dot_general(h, w, (((1,), (0,)), ((), ())), preferred_element_type=F32)
                if light:
                    ring[hd, pl.ds(ppos, LT), :] = qkv[M:]
                    qkvs[hd] = qkv[0:M]
                else:
                    qkvs[hd] = qkv

            pref = {}

            def prefetch(i):
                for kind, a in SCHED[i + 1:]:
                    if kind == "q":
                        break
                    for j in {"s": (0, 1), "p": (2,), "w": ()}[kind]:
                        if (a, j) in pref or a not in qkvs:
                            continue
                        pref[a, j] = ring[a, pl.ds(apos, SEG), j * E:(j + 1) * E]

            def part(hd, j):
                v = qkvs[hd][:, j * E:(j + 1) * E]
                if light:
                    v = jnp.concatenate([v, pref[hd, j]], axis=0)
                return v

            def st_s(hd):
                q = _rb(part(hd, 0))
                k = part(hd, 1).astype(BF16)
                sc = lax.dot_general(q, k, (((1,), (1,)), ((), ())), preferred_element_type=F32)
                sc = jnp.where(mask, sc, NEG / scale)
                mx = jnp.max(sc, axis=-1, keepdims=True)
                e = jnp.exp2((sc - mx) * (scale * LOG2E))
                ps[hd] = (_rb(e), 1.0 / jnp.sum(e, axis=-1, keepdims=True))

            def st_pv(hd):
                e, inv = ps[hd]
                v = part(hd, 2).astype(BF16)
                pv = lax.dot_general(e, v, (((1,), (0,)), ((), ())), preferred_element_type=F32)
                os_[hd] = _rb(pv * inv)

            def st_wo(h0, n, acc):
                o = jnp.concatenate([os_[h0 + j] for j in range(n)], axis=1)
                part = jnp.concatenate(
                    [_mm(o, pltpu.bitcast(wo[j, h0 * E // 2:(h0 + n) * E // 2, :], BF16)) for j in range(ND)], axis=1)
                return part if acc is None else acc + part

            for i, (kind, a) in enumerate(SCHED):
                if kind == "q":
                    if a == A_POST:
                        top = post(s - PL, top)
                    if a == A_POST + A_D:
                        wqkv[anchor, 256:264, 0:128] = pltpu.bitcast(jnp.broadcast_to(top[0] + top[2], (8, 128)), I32)
                    if light:
                        prefetch(i)
                    st_qkv(a)
                    if light and a == H - 1:
                        prefetch(i)
                elif kind == "s":
                    st_s(a)
                elif kind == "p":
                    st_pv(a)
                else:
                    acc = st_wo(a[0], a[1], acc)
            if light:
                sn = pl.multiple_of(T + jnp.minimum(s + 1, NL - 1) * LT, 8)
            else:
                sn = pl.multiple_of(jnp.minimum(s + 1, NSEG - 1) * SEG, SEG)
            hbuf[M:M + nt, :] = pre(xbuf[pl.ds(sn, nt), :])
            acc = _rb(acc)
            hbuf[0:M, :] = acc[0:M]
            abuf[pl.ds(pl.multiple_of(s * SEG, SEG), SEG), :] = acc[M:L].astype(BF16)

            @pl.when(s >= PL)
            def _():
                out_copy(s - PL).start()
            return top

        ninf = jnp.full((8, 1), -jnp.inf, F32)
        izero = jnp.zeros((8, 1), I32)
        with _sc("m1_light"):
            top = lax.fori_loop(0, NL, functools.partial(step, light=True), (ninf, izero, ninf, izero))
        hbuf[M:L, :] = pre(xbuf[NL * SEG:(NL + 1) * SEG, :])
        with _sc("m2_normal"):
            top = lax.fori_loop(NL, NRUN, functools.partial(step, light=False), top)
        for sp in range(NSEG - PL, NSEG):
            top = post(sp, top)
            out_copy(sp).start()

        b1, i1v, b2, i2v = top
        m1 = jnp.max(b1)
        i1 = jnp.min(jnp.where(b1 == m1, i1v, S))
        win = (b1 == m1) & (i1v == i1)
        c1 = jnp.where(win, b2, b1)
        ci = jnp.where(win, i2v, i1v)
        m2 = jnp.max(c1)
        i2 = jnp.min(jnp.where(c1 == m2, ci, S))
        i1 = jnp.clip(i1, 0, S - 1)
        i2 = jnp.clip(i2, 0, S - 1)

        rows = []
        for n, ii in enumerate((i1, i2)):
            b = pl.multiple_of((ii // 16) * 16, 16)
            gidx = b + lax.broadcasted_iota(I32, (16, D), 0)
            x1, h2 = residual(xbuf[pl.ds(b, 16), :], abuf[pl.ds(b, 16), :])
            hit = gidx == ii
            x1 = jnp.sum(jnp.where(hit, x1, 0.0), axis=0, keepdims=True)
            h2 = jnp.sum(jnp.where(hit, h2, 0.0), axis=0, keepdims=True)
            sel[n:n + 1, :] = h2
            rows.append((b, x1, h2))
        xs = sel[...]
        wait(cp_ffn)
        acts = []
        for j in range(NF):
            gq = _rb(_mm(xs, pltpu.bitcast(wg[j], BF16)))
            uq = _rb(_mm(xs, pltpu.bitcast(wu[j], BF16)))
            acts.append(_rb(_rb(gq * jax.nn.sigmoid(gq)) * uq))
        act = jnp.concatenate(acts, axis=1)
        y = _rb(jnp.concatenate([_mm(act, pltpu.bitcast(wd[j], BF16)) for j in range(ND)], axis=1))
        new = []
        for n, mm in enumerate((m1, m2)):
            _, x1, h2 = rows[n]
            sig = _rb(jax.nn.sigmoid(jnp.full((1, D), mm, F32)))
            new.append(x1 + modbuf[5, 0:1, :] * (h2 + _rb(y[n:n + 1] * sig)))
        for n in range(2):
            b = rows[n][0]
            gidx = b + lax.broadcasted_iota(I32, (16, D), 0)
            blk = outbuf[pl.ds(b + PL * SEG, 16), :].astype(F32)
            blk = jnp.where(gidx == i1, new[0], jnp.where(gidx == i2, new[1], blk))
            fixbuf[n] = blk.astype(BF16)
        pltpu.make_async_copy(outbuf.at[pl.ds(PL * SEG, NRUN * SEG), :], out_hbm.at[pl.ds(0, NRUN * SEG), :], sems.at[12]).wait()
        for n in range(2):
            cp = pltpu.make_async_copy(fixbuf.at[n], out_hbm.at[pl.ds(rows[n][0], 16), :], sems.at[13])
            cp.start()
            cp.wait()

    any_spec = pl.BlockSpec(memory_space=pl.ANY)
    vmem_spec = pl.BlockSpec(memory_space=pltpu.VMEM)
    return pl.pallas_call(
        kernel,
        out_shape=jax.ShapeDtypeStruct((S, D), BF16),
        in_specs=[any_spec, vmem_spec, any_spec, any_spec, any_spec, any_spec, vmem_spec,
                  any_spec, any_spec, any_spec, vmem_spec, any_spec],
        out_specs=any_spec,
        scratch_shapes=[
            pltpu.VMEM((H + 1, D // 2, 3 * E), I32),
            pltpu.VMEM((ND, H * E // 2, 128), I32),
            pltpu.VMEM((6 * ND, D // 2, 128), I32),
            pltpu.VMEM((NF, D // 2, 128), I32),
            pltpu.VMEM((NF, D // 2, 128), I32),
            pltpu.VMEM((ND, FF // 2, 128), I32),
            pltpu.VMEM((2, 3, D, HG, E), BF16),
            pltpu.VMEM((S, D), BF16),
            pltpu.VMEM((S, D), BF16),
            pltpu.VMEM((S + PL * SEG, D), BF16),
            pltpu.VMEM((L, D), F32),
            pltpu.VMEM((6, 8, D), F32),
            pltpu.VMEM((8, D), F32),
            pltpu.VMEM((8, D), F32),
            pltpu.VMEM((2, 16, D), BF16),
            pltpu.VMEM((H, R, 3 * E), F32),
            pltpu.VMEM((T, D), BF16),
            pltpu.SMEM((1,), I32),
            pltpu.SemaphoreType.DMA((16,)),
        ],
        compiler_params=pltpu.CompilerParams(vmem_limit_bytes=120 * 1024 * 1024),
        name="adaln_rmt_mod",
    )


@functools.partial(jax.jit, static_argnames=("A_seg_len",))
def pallas_adaLN_cond__memory_aug_recurrent_mem_tr__moe_arch_mod__prompt_kernel(
    A_x: jax.Array,
    A_mem0: jax.Array,
    A_Wq: jax.Array,
    A_Wk: jax.Array,
    A_Wv: jax.Array,
    A_Wo: jax.Array,
    A_seg_len: int,
    B_x: jax.Array,
    B_w_r: jax.Array,
    B_w_gate: jax.Array,
    B_w_up: jax.Array,
    B_w_down: jax.Array,
    c: jax.Array,
    w_mod: jax.Array,
):
    del B_x
    B, S, D = A_x.shape
    H, E = A_Wq.shape[1], A_Wq.shape[2]
    M = A_mem0.shape[1]
    SEG = int(A_seg_len)
    FF = B_w_gate.shape[1]
    assert B == 1 and S % SEG == 0
    call = _build(S, D, H, E, M, SEG, FF)
    out = call(
        A_x.reshape(S, D), A_mem0, A_Wq, A_Wk, A_Wv, A_Wo.reshape(H * E, D),
        B_w_r, B_w_gate, B_w_up, B_w_down, c, w_mod,
    )
    return out.reshape(B, S, D)
```

```python
import functools

import jax
import jax.numpy as jnp
from jax import lax
import jax.experimental.pallas as pl
import jax.experimental.pallas.tpu as pltpu

LS, LP, LW = [int(v) for v in '1,3,5'.split(',')]
F32 = jnp.float32
import contextlib
_sc = lambda n: contextlib.nullcontext()
BF16 = jnp.bfloat16
I32 = jnp.int32
EPS = 1e-5
NEG = -1000000000.0
LOG2E = 1.4426950408889634


def _rb(v):
    return v.astype(BF16).astype(F32)


def _layernorm(x):
    m = jnp.mean(x, axis=-1, keepdims=True)
    d = x - m
    v = jnp.mean(d * d, axis=-1, keepdims=True)
    return d * lax.rsqrt(v + EPS)


def _mm(a, b):
    return lax.dot_general(a, b, (((1,), (0,)), ((), ())), preferred_element_type=F32)


def _mm_nt(a, b):
    return lax.dot_general(a, b, (((1,), (1,)), ((), ())), preferred_element_type=F32)


def _transpose4(v):
    sub = lax.broadcasted_iota(I32, (8, 128), 0)
    v = list(v)
    for k in (2, 1):
        m = (sub & k) != 0
        for i in range(4):
            if i & k:
                continue
            a, b = v[i], v[i + k]
            v[i] = jnp.where(m, pltpu.roll(b, k, 0), a)
            v[i + k] = jnp.where(m, b, pltpu.roll(a, 8 - k, 0))
    return v


def _build(S, D, H, E, M, SEG, FF):
    NSEG = S // SEG
    L = M + SEG
    HG = 8
    NG = H // HG
    WG = 4
    scale = float(E) ** (-0.5)

    NRUN = int(NSEG)
    LT = 24
    NL = int(30)
    T = NL * (SEG - LT)
    R = 288
    assert T % LT == 0 and R % LT == 0 and R % SEG == 0 and R >= T + LT and T % 16 == 0
    XA = -(-(T + 3 * LT) // 16) * 16
    ND = D // 128
    NF = FF // 128
    WOG = [int(v) for v in '4,4,4,4,4,4,4,3,1'.split(',')] if H == 32 else [H]
    SCHED = []
    ends = {}
    h0 = 0
    for n in WOG:
        ends[h0 + n - 1] = (h0, n)
        h0 += n
    for t in range(H + LW):
        if t < H:
            SCHED.append(("q", t))
        if 0 <= t - LS < H:
            SCHED.append(("s", t - LS))
        if 0 <= t - LP < H:
            SCHED.append(("p", t - LP))
        if t - LW in ends:
            SCHED.append(("w", ends[t - LW]))
    if H == 32:
        cut = SCHED.index(("q", 31)) + 1
        head = [e for e in SCHED[:cut]]
        tail = []
        for tok in "s30 p28 p29 w24:1 s31 w25:2 p30 w27:1 p31 w28:2 w30:1 w31:1".split():
            if tok[0] in "ps":
                tail.append((tok[0], int(tok[1:])))
            else:
                a, b = tok[1:].split(":")
                tail.append(("w", (int(a), int(b))))
        done = {e for e in head}
        head = [e for e in head if e not in tail]
        SCHED = head + tail
    A_POST, A_PRE, A_D = [int(v) for v in '2,0,4'.split(',')]
    REST_STEP = 2
    PL = 2

    def kernel(x_hbm, mem0_ref, wq_hbm, wk_hbm, wv_hbm, wo_hbm, wr_ref, wg_hbm, wu_hbm, wd_hbm,
               c_ref, wmod_hbm, out_hbm,
               wqkv, wo, wmod, wg, wu, wd, stg,
               xbuf, abuf, outbuf, hbuf, modbuf, wrbuf, sel, fixbuf, ring, hT, zs, sems):

        def slab_copies(src, dst, js, sem):
            return [pltpu.make_async_copy(src.at[:, pl.ds(j * 128, 128)], dst.at[j].bitcast(BF16), sem)
                    for j in js]

        def start(cps):
            for cp in cps:
                cp.start()

        def wait(cps):
            for cp in cps:
                cp.wait()

        cp_mod0 = slab_copies(wmod_hbm, wmod, range(0, 2 * ND), sems.at[0])
        cp_mod1 = slab_copies(wmod_hbm, wmod, range(2 * ND, 6 * ND), sems.at[1])
        cp_xa = [pltpu.make_async_copy(x_hbm.at[pl.ds(0, XA), :], xbuf.at[pl.ds(0, XA), :], sems.at[2])]
        cp_xb = [pltpu.make_async_copy(x_hbm.at[pl.ds(XA, S - XA), :], xbuf.at[pl.ds(XA, S - XA), :], sems.at[3])]
        cp_wo = slab_copies(wo_hbm, wo, range(ND), sems.at[4])
        cp_ffn = (slab_copies(wg_hbm, wg, range(NF), sems.at[5]) + slab_copies(wu_hbm, wu, range(NF), sems.at[5])
                  + slab_copies(wd_hbm, wd, range(ND), sems.at[5]))

        def wcopies(g):
            slot = g % 2
            hs = pl.ds(pl.multiple_of(g * HG, HG), HG)
            return [pltpu.make_async_copy(w.at[:, hs, :], stg.at[slot, j], sems.at[6 + 3 * slot + j])
                    for j, w in enumerate((wq_hbm, wk_hbm, wv_hbm))]

        def mod_vectors(js):
            cv = c_ref[...].astype(F32)
            sc8 = jnp.broadcast_to(_rb(cv * jax.nn.sigmoid(cv)), (8, D))
            for j in js:
                mj = jnp.concatenate(
                    [_mm(sc8, pltpu.bitcast(wmod[j * ND + n], BF16)) for n in range(ND)], axis=1)
                mj = _rb(mj)
                modbuf[j] = (1.0 + mj) if j in (1, 4) else mj

        def pre(xs):
            return _rb(_layernorm(xs.astype(F32)) * modbuf[1, 0:1, :] + modbuf[0, 0:1, :])

        zs[0] = 0
        start(cp_mod0)
        start(cp_xa)
        start(wcopies(0))
        start(wcopies(1))
        wrbuf[...] = jnp.broadcast_to(wr_ref[...].astype(F32).reshape(1, D), (8, D))
        sel[...] = jnp.zeros((8, D), F32)
        hbuf[0:M, :] = mem0_ref[0].astype(F32)
        with _sc("p0_waitmod"):
            wait(cp_mod0)
        mod_vectors((0, 1))
        wait(cp_xa)

        def pre_loop(i, carry):
            r0 = pl.multiple_of(i * 48, 16)
            hT[pl.ds(r0, 48), :] = pre(xbuf[pl.ds(r0, 48), :]).astype(BF16)
            return carry

        lax.fori_loop(0, T // 48, pre_loop, 0)
        hbuf[M:M + LT, :] = pre(xbuf[T:T + LT, :])

        def relayout(g, j, d0):
            d0 = pl.multiple_of(d0, 16)
            blk = stg[g % 2, j, pl.ds(d0, 16)]
            ev, od = [
                _transpose4([pltpu.bitcast(jnp.concatenate([blk[2 * a + p], blk[2 * a + p + 8]], axis=0), I32)
                             for a in range(4)]) for p in (0, 1)]
            rows = pl.ds(pl.multiple_of(d0 // 2, 8), 8)
            cols = pl.ds(pl.multiple_of(j * E, E), E)
            for hp in range(HG // 2):
                wqkv[g * HG + 2 * hp, rows, cols] = (ev[hp] & 0xFFFF) | (od[hp] << 16)
                wqkv[g * HG + 2 * hp + 1, rows, cols] = (
                    lax.shift_right_logical(ev[hp], 16) | (od[hp] & jnp.int32(-65536)))

        def project(hd):
            ring[hd, 0:T, :] = _mm(hT[...], pltpu.bitcast(wqkv[hd], BF16))

        def project_pair(i, carry):
            project(2 * i)
            project(2 * i + 1)
            return carry

        cp0 = wcopies(0)
        with _sc("p1_first"):
            for j in range(3):
                cp0[j].wait()

                def rl(i, carry, j=j):
                    relayout(0, j, i * 32)
                    relayout(0, j, i * 32 + 16)
                    return carry

                lax.fori_loop(0, D // 32, rl, 0)
        start(wcopies(2))

        def group(g, carry):
            project_pair(g * (HG // 2), 0)

            def fused(j, carry):
                pltpu.make_async_copy(wq_hbm.at[:, pl.ds(0, HG), :], stg.at[(g + 1) % 2, j],
                                      sems.at[6 + 3 * ((g + 1) % 2) + j]).wait()

                def inner(u, carry):
                    project(g * HG + 2 + 2 * j + u)
                    for w in range(D // 32):
                        relayout(g + 1, j, u * (D // 2) + w * 16)
                    return carry

                return lax.fori_loop(0, 2, inner, carry)

            lax.fori_loop(0, 3, fused, 0)

            @pl.when(g == 0)
            def _():
                start(wcopies(3))
                start(cp_wo)
                start(cp_mod1)
                start(cp_xb)
            return carry

        assert NG == 4 and HG == 8
        with _sc("p3_project"):
            lax.fori_loop(0, NG - 1, group, 0)
            lax.fori_loop(H // 2 - HG // 2, H // 2, project_pair, 0)
        with _sc("p4_waitwo"):
            wait(cp_wo)

        row = lax.broadcasted_iota(I32, (L, L), 0)
        col = lax.broadcasted_iota(I32, (L, L), 1)
        mask = (row < M) | (row >= col)

        def second_half():
            wait(cp_mod1)
            wait(cp_xb)
            start(cp_ffn)
            mod_vectors((2, 3, 4, 5))

        def residual(xs, a):
            x1 = xs.astype(F32) + modbuf[2, 0:1, :] * a.astype(F32)
            h2 = _rb(_layernorm(x1) * modbuf[4, 0:1, :] + modbuf[3, 0:1, :])
            return x1, h2

        def out_copy(sp):
            dst = pl.multiple_of(jnp.maximum(sp, 0) * SEG, SEG)
            src = pl.multiple_of((sp + PL) * SEG, SEG)
            return pltpu.make_async_copy(outbuf.at[pl.ds(src, SEG), :], out_hbm.at[pl.ds(dst, SEG), :], sems.at[12])

        def post(sp, top):
            src = pl.multiple_of(jnp.maximum(sp, 0) * SEG, SEG)
            dst = pl.multiple_of((sp + PL) * SEG, SEG)
            a = jnp.where(sp >= 0, abuf[pl.ds(src, SEG), :].astype(F32), 0.0)
            x1, h2 = residual(xbuf[pl.ds(src, SEG), :], a)
            outbuf[pl.ds(dst, SEG), :] = (x1 + modbuf[5, 0:1, :] * h2).astype(BF16)
            r = _rb(jnp.sum(h2 * wrbuf[0:1, :], axis=-1, keepdims=True))
            r = jnp.where(sp >= 0, r, -jnp.inf)
            b1, i1, b2, i2 = top
            sub = lax.broadcasted_iota(I32, (8, 1), 0)
            for t in range(SEG // 8):
                rv = r[t * 8:(t + 1) * 8]
                iv = src + t * 8 + sub
                g1 = rv > b1
                g2 = rv > b2
                b2 = jnp.where(g1, b1, jnp.where(g2, rv, b2))
                i2 = jnp.where(g1, i1, jnp.where(g2, iv, i2))
                b1 = jnp.where(g1, rv, b1)
                i1 = jnp.where(g1, iv, i1)
            return b1, i1, b2, i2

        def step(s, top, light):
            if light:
                pl.when(s == REST_STEP)(second_half)
            nt = LT if light else SEG
            anchor = H + zs[0]
            h = hbuf[0:M + nt, :]
            acc = None
            qkvs, ps, os_ = {}, {}, {}
            if light:
                ppos = pl.multiple_of(lax.rem(T + s * LT, R), 8)
                apos = pl.multiple_of(lax.rem(s * SEG, R), SEG)

            def st_qkv(hd):
                w = pltpu.bitcast(wqkv[hd], BF16)
                qkv = lax.dot_general(h, w, (((1,), (0,)), ((), ())), preferred_element_type=F32)
                if light:
                    ring[hd, pl.ds(ppos, LT), :] = qkv[M:]
                    qkvs[hd] = qkv[0:M]
                else:
                    qkvs[hd] = qkv

            pref = {}

            def prefetch(i):
                for kind, a in SCHED[i + 1:]:
                    if kind == "q":
                        break
                    for j in {"s": (0, 1), "p": (2,), "w": ()}[kind]:
                        if (a, j) in pref or a not in qkvs:
                            continue
                        pref[a, j] = ring[a, pl.ds(apos, SEG), j * E:(j + 1) * E]

            def part(hd, j):
                v = qkvs[hd][:, j * E:(j + 1) * E]
                if light:
                    v = jnp.concatenate([v, pref[hd, j]], axis=0)
                return v

            def st_s(hd):
                q = _rb(part(hd, 0))
                k = part(hd, 1).astype(BF16)
                sc = lax.dot_general(q, k, (((1,), (1,)), ((), ())), preferred_element_type=F32)
                sc = jnp.where(mask, sc, NEG / scale)
                mx = jnp.max(sc, axis=-1, keepdims=True)
                e = jnp.exp2((sc - mx) * (scale * LOG2E))
                ps[hd] = (_rb(e), 1.0 / jnp.sum(e, axis=-1, keepdims=True))

            def st_pv(hd):
                e, inv = ps[hd]
                v = part(hd, 2).astype(BF16)
                pv = lax.dot_general(e, v, (((1,), (0,)), ((), ())), preferred_element_type=F32)
                os_[hd] = _rb(pv * inv)

            def st_wo(h0, n, acc):
                o = jnp.concatenate([os_[h0 + j] for j in range(n)], axis=1)
                part = jnp.concatenate(
                    [_mm(o, pltpu.bitcast(wo[j, h0 * E // 2:(h0 + n) * E // 2, :], BF16)) for j in range(ND)], axis=1)
                return part if acc is None else acc + part

            for i, (kind, a) in enumerate(SCHED):
                if kind == "q":
                    if a == A_POST:
                        top = post(s - PL, top)
                    if a == A_POST + A_D:
                        wqkv[anchor, 256:264, 0:128] = pltpu.bitcast(jnp.broadcast_to(top[0] + top[2], (8, 128)), I32)
                    if light:
                        prefetch(i)
                    st_qkv(a)
                    if light and a == H - 1:
                        prefetch(i)
                elif kind == "s":
                    st_s(a)
                elif kind == "p":
                    st_pv(a)
                else:
                    acc = st_wo(a[0], a[1], acc)
            if light:
                sn = pl.multiple_of(T + jnp.minimum(s + 1, NL - 1) * LT, 8)
            else:
                sn = pl.multiple_of(jnp.minimum(s + 1, NSEG - 1) * SEG, SEG)
            hbuf[M:M + nt, :] = pre(xbuf[pl.ds(sn, nt), :])
            acc = _rb(acc)
            hbuf[0:M, :] = acc[0:M]
            abuf[pl.ds(pl.multiple_of(s * SEG, SEG), SEG), :] = acc[M:L].astype(BF16)

            @pl.when(s >= PL)
            def _():
                out_copy(s - PL).start()
            return top

        ninf = jnp.full((8, 1), -jnp.inf, F32)
        izero = jnp.zeros((8, 1), I32)
        with _sc("m1_light"):
            top = lax.fori_loop(0, NL, functools.partial(step, light=True), (ninf, izero, ninf, izero))
        hbuf[M:L, :] = pre(xbuf[NL * SEG:(NL + 1) * SEG, :])
        with _sc("m2_normal"):
            top = lax.fori_loop(NL, NRUN, functools.partial(step, light=False), top)
        for sp in range(NSEG - PL, NSEG):
            top = post(sp, top)
            out_copy(sp).start()

        b1, i1v, b2, i2v = top
        m1 = jnp.max(b1)
        i1 = jnp.min(jnp.where(b1 == m1, i1v, S))
        win = (b1 == m1) & (i1v == i1)
        c1 = jnp.where(win, b2, b1)
        ci = jnp.where(win, i2v, i1v)
        m2 = jnp.max(c1)
        i2 = jnp.min(jnp.where(c1 == m2, ci, S))
        i1 = jnp.clip(i1, 0, S - 1)
        i2 = jnp.clip(i2, 0, S - 1)

        rows = []
        for n, ii in enumerate((i1, i2)):
            b = pl.multiple_of((ii // 16) * 16, 16)
            gidx = b + lax.broadcasted_iota(I32, (16, D), 0)
            x1, h2 = residual(xbuf[pl.ds(b, 16), :], abuf[pl.ds(b, 16), :])
            hit = gidx == ii
            x1 = jnp.sum(jnp.where(hit, x1, 0.0), axis=0, keepdims=True)
            h2 = jnp.sum(jnp.where(hit, h2, 0.0), axis=0, keepdims=True)
            sel[n:n + 1, :] = h2
            rows.append((b, x1, h2))
        xs = sel[...]
        wait(cp_ffn)
        acts = []
        for j in range(NF):
            gq = _rb(_mm(xs, pltpu.bitcast(wg[j], BF16)))
            uq = _rb(_mm(xs, pltpu.bitcast(wu[j], BF16)))
            acts.append(_rb(_rb(gq * jax.nn.sigmoid(gq)) * uq))
        act = jnp.concatenate(acts, axis=1)
        y = _rb(jnp.concatenate([_mm(act, pltpu.bitcast(wd[j], BF16)) for j in range(ND)], axis=1))
        new = []
        for n, mm in enumerate((m1, m2)):
            _, x1, h2 = rows[n]
            sig = _rb(jax.nn.sigmoid(jnp.full((1, D), mm, F32)))
            new.append(x1 + modbuf[5, 0:1, :] * (h2 + _rb(y[n:n + 1] * sig)))
        for n in range(2):
            b = rows[n][0]
            gidx = b + lax.broadcasted_iota(I32, (16, D), 0)
            blk = outbuf[pl.ds(b + PL * SEG, 16), :].astype(F32)
            blk = jnp.where(gidx == i1, new[0], jnp.where(gidx == i2, new[1], blk))
            fixbuf[n] = blk.astype(BF16)
        pltpu.make_async_copy(outbuf.at[pl.ds(PL * SEG, NRUN * SEG), :], out_hbm.at[pl.ds(0, NRUN * SEG), :], sems.at[12]).wait()
        for n in range(2):
            cp = pltpu.make_async_copy(fixbuf.at[n], out_hbm.at[pl.ds(rows[n][0], 16), :], sems.at[13])
            cp.start()
            cp.wait()

    any_spec = pl.BlockSpec(memory_space=pl.ANY)
    vmem_spec = pl.BlockSpec(memory_space=pltpu.VMEM)
    return pl.pallas_call(
        kernel,
        out_shape=jax.ShapeDtypeStruct((S, D), BF16),
        in_specs=[any_spec, vmem_spec, any_spec, any_spec, any_spec, any_spec, vmem_spec,
                  any_spec, any_spec, any_spec, vmem_spec, any_spec],
        out_specs=any_spec,
        scratch_shapes=[
            pltpu.VMEM((H + 1, D // 2, 3 * E), I32),
            pltpu.VMEM((ND, H * E // 2, 128), I32),
            pltpu.VMEM((6 * ND, D // 2, 128), I32),
            pltpu.VMEM((NF, D // 2, 128), I32),
            pltpu.VMEM((NF, D // 2, 128), I32),
            pltpu.VMEM((ND, FF // 2, 128), I32),
            pltpu.VMEM((2, 3, D, HG, E), BF16),
            pltpu.VMEM((S, D), BF16),
            pltpu.VMEM((S, D), BF16),
            pltpu.VMEM((S + PL * SEG, D), BF16),
            pltpu.VMEM((L, D), F32),
            pltpu.VMEM((6, 8, D), F32),
            pltpu.VMEM((8, D), F32),
            pltpu.VMEM((8, D), F32),
            pltpu.VMEM((2, 16, D), BF16),
            pltpu.VMEM((H, R, 3 * E), F32),
            pltpu.VMEM((T, D), BF16),
            pltpu.SMEM((1,), I32),
            pltpu.SemaphoreType.DMA((16,)),
        ],
        compiler_params=pltpu.CompilerParams(vmem_limit_bytes=120 * 1024 * 1024),
        name="adaln_rmt_mod",
    )


@functools.partial(jax.jit, static_argnames=("A_seg_len",))
def pallas_adaLN_cond__memory_aug_recurrent_mem_tr__moe_arch_mod__prompt_kernel(
    A_x: jax.Array,
    A_mem0: jax.Array,
    A_Wq: jax.Array,
    A_Wk: jax.Array,
    A_Wv: jax.Array,
    A_Wo: jax.Array,
    A_seg_len: int,
    B_x: jax.Array,
    B_w_r: jax.Array,
    B_w_gate: jax.Array,
    B_w_up: jax.Array,
    B_w_down: jax.Array,
    c: jax.Array,
    w_mod: jax.Array,
):
    del B_x
    B, S, D = A_x.shape
    H, E = A_Wq.shape[1], A_Wq.shape[2]
    M = A_mem0.shape[1]
    SEG = int(A_seg_len)
    FF = B_w_gate.shape[1]
    assert B == 1 and S % SEG == 0
    call = _build(S, D, H, E, M, SEG, FF)
    out = call(
        A_x.reshape(S, D), A_mem0, A_Wq, A_Wk, A_Wv, A_Wo.reshape(H * E, D),
        B_w_r, B_w_gate, B_w_up, B_w_down, c, w_mod,
    )
    return out.reshape(B, S, D)
```
